```python
import os as _os
_os.environ.setdefault("JAX_PLATFORMS", "cpu")
import jax
import jax.numpy as jnp

def _softmax(x, axis=-1):
    return jax.nn.softmax(x, axis=axis)
def _gelu(x):
    return jax.nn.gelu(x, approximate=True)
def _silu(x):
    return jax.nn.silu(x)
def _sigmoid(x):
    return jax.nn.sigmoid(x)
def _layernorm(x, axis=-1, eps=1e-5):
    m = jnp.mean(x, axis=axis, keepdims=True)
    v = jnp.var(x, axis=axis, keepdims=True)
    return (x - m) / jnp.sqrt(v + eps)
def _scatter_add(tgt, idx, src, axis=0):
    return tgt.at[idx].add(src)
def _segment_sum(src, seg, n):
    return jax.ops.segment_sum(src, seg, n)
class _Rng:
    def __init__(self, key):
        self._k = key
    def _next(self):
        self._k, sub = jax.random.split(self._k)
        return sub
    def normal(self, shape):
        return jax.random.normal(self._next(), shape, dtype=jnp.bfloat16)
    def randint(self, lo, hi, shape):
        return jax.random.randint(self._next(), shape, lo, hi, dtype=jnp.int32)
    def uniform(self, shape, lo=0.0, hi=1.0):
        return jax.random.uniform(self._next(), shape, jnp.bfloat16, lo, hi)
    def permutation(self, n):
        return jax.random.permutation(self._next(), n)


kernel_name = 'interleave_layers__linear_kernel_hedgehog__dense_activation_silu__prompt'

def setup_inputs():
    _rng = _Rng(jax.random.key(int.from_bytes(__import__("os").urandom(4), "little")))
    _w = (lambda a: (lambda t: t.astype(jnp.bfloat16) if jnp.issubdtype(t.dtype, jnp.floating) else t)(jnp.asarray(a)))
    def _A_setup():
        B, S, D, H = 1, 2048, 640, 32
        Dh = D // H
        return {
            "x": _w((lambda *s: _rng.normal(s) * 0.05)(B, S, D)),
            "wqkv": _w((lambda *s: _rng.normal(s) * 0.4)(D, 3 * D)),
            "w_phi": _w((lambda *s: _rng.normal(s) * 0.4)(H, Dh, Dh) * (Dh ** -0.5)),
            "wo": _w((lambda *s: _rng.normal(s) * 0.05)(D, D)),
        }
    _A_in = _A_setup()

    def _B_setup():
        B, S, D, F = 1, 2048, 640, 1728
        return {
            "x": _w((lambda *s: _rng.normal(s) * 0.05)(B, S, D)),
            "w1": _w((lambda *s: _rng.normal(s) * 1.6)(D, F) * (D ** -0.5)),
            "w2": _w((lambda *s: _rng.normal(s) * 1.6)(F, D) * (F ** -0.5)),
        }
    _B_in = _B_setup()

    return {
        "A_x": _A_in["x"],
        "A_wqkv": _A_in["wqkv"],
        "A_w_phi": _A_in["w_phi"],
        "A_wo": _A_in["wo"],
        "B_x": _B_in["x"],
        "B_w1": _B_in["w1"],
        "B_w2": _B_in["w2"],
    }

def reference(A_x, A_wqkv, A_w_phi, A_wo, B_x, B_w1, B_w2):
    def _A_ref(x, wqkv, w_phi, wo):
        B, S, D = x.shape
        H = 32; Dh = D // H
        qkv = (lambda x, *d: x.transpose(*d))((x @ wqkv).reshape(B, S, 3, H, Dh), 2, 0, 3, 1, 4)
        q, k, v = qkv[0], qkv[1], qkv[2]
        pq = jnp.einsum("bhsd,hdf->bhsf", q, w_phi)
        pk = jnp.einsum("bhsd,hdf->bhsf", k, w_phi)
        phi_q = jnp.concatenate([_softmax(pq, axis=-1), _softmax(-pq, axis=-1)], axis=-1)
        phi_k = jnp.concatenate([_softmax(pk, axis=-1), _softmax(-pk, axis=-1)], axis=-1)
        kv = jnp.einsum("bhsf,bhsd->bhfd", phi_k, v)
        z  = jnp.einsum("bhsf->bhf", phi_k)
        num = jnp.einsum("bhqf,bhfd->bhqd", phi_q, kv)
        den = jnp.einsum("bhqf,bhf->bhq", phi_q, z)[..., None] + 1e-6
        o = num / den
        return (lambda x, *d: x.transpose(*d))(o, 0, 2, 1, 3).reshape(B, S, D) @ wo

    def _B_ref(x, w1, w2):
        h = jnp.einsum("bsd,df->bsf", x, w1)
        h = _silu(h)
        out = jnp.einsum("bsf,fd->bsd", h, w2)
        return out

    x = A_x
    x = x + _A_ref(_layernorm(x, axis=-1), A_wqkv, A_w_phi, A_wo)
    x = x + _B_ref(_layernorm(x, axis=-1), B_w1, B_w2)
    x = x + _A_ref(_layernorm(x, axis=-1), A_wqkv, A_w_phi, A_wo)
    x = x + _B_ref(_layernorm(x, axis=-1), B_w1, B_w2)
    return x
```

```python
import jax
import jax.numpy as jnp
from jax import lax
import jax.experimental.pallas as pl
import jax.experimental.pallas.tpu as pltpu

S, D, H, DH, F = 2048, 640, 32, 20, 1728
G = 16
T = 256
NW1 = 2
MS = 2
NSM = 8
NKV = 2
GPP = 2
FC = 384
XD, GAP, GAP2, GAP3 = 0.5, 0.8, 0.3, 0.8
HT0, HDT = 0.6, 0.05
LOG2E = 1.4426950408889634
NT = (((1,), (1,)), ((), ()))
TN = (((0,), (0,)), ((), ()))
f32, bf16, u32, i32 = jnp.float32, jnp.bfloat16, jnp.uint32, jnp.int32


def _ln(x):
    m = jnp.mean(x, axis=-1, keepdims=True)
    xc = x - m
    v = jnp.mean(xc * xc, axis=-1, keepdims=True)
    return pltpu.bitcast((xc * lax.rsqrt(v + 1e-5)).astype(bf16), u32)


def _pack(a, b):
    return pltpu.bitcast(pltpu.pack_elementwise([a, b], packed_dtype=bf16), u32)


def _rcp(x):
    r = pl.reciprocal(x, approx=True)
    return r * (2.0 - x * r)


def _tree(op, xs):
    while len(xs) > 1:
        xs = [op(xs[i], xs[i + 1]) if i + 1 < len(xs) else xs[i] for i in range(0, len(xs), 2)]
    return xs[0]


def _b(x):
    return pltpu.bitcast(x, bf16)


def kernel(x_hbm, wqkv_hbm, wphi_hbm, wo_hbm, w1t_hbm, w2_hbm, o_hbm,
           x_ref, wqkv_ref, wphi_ref, wo_ref, w1t_ref, w2_ref, wc_ref,
           xs_ref, y1_ref, y2_ref, wt_ref, phiq_ref, phik_ref, kv_ref, kvb_ref,
           wsem, xsem, osem):
    NC = T // 128
    NTILE = S // T

    def rows(t):
        return slice(t * T, (t + 1) * T)

    def hrows(t):
        return slice(t * T // 2, (t + 1) * T // 2)

    def x_copy(t):
        return pltpu.make_async_copy(x_hbm.at[rows(t)], x_ref.at[rows(t)], xsem.at[t])

    def o_copy(t):
        return pltpu.make_async_copy(x_ref.at[rows(t)], o_hbm.at[rows(t)], osem.at[t])

    wq_u32 = wqkv_hbm.bitcast(u32)
    c_phi = pltpu.make_async_copy(wphi_hbm, wphi_ref, wsem.at[0])
    c_part = [pltpu.make_async_copy(wq_u32.at[:, p * D:(p + 1) * D], wqkv_ref.at[:, p * D:(p + 1) * D], wsem.at[1 + p])
              for p in range(3)]
    c_wo = pltpu.make_async_copy(wo_hbm.bitcast(u32), wo_ref, wsem.at[4])
    c_w1 = pltpu.make_async_copy(w1t_hbm.bitcast(u32), w1t_ref, wsem.at[5])
    c_w2 = pltpu.make_async_copy(w2_hbm.bitcast(u32), w2_ref, wsem.at[6])
    c_phi.start()
    c_part[1].start()
    for t in range(NW1):
        x_copy(t).start()

    eye = jnp.where(lax.broadcasted_iota(i32, (H, H), 0) == lax.broadcasted_iota(i32, (H, H), 1), 1.0, 0.0).astype(bf16)
    oh = jnp.where((lax.broadcasted_iota(i32, (160, 128), 0) >> 3) == lax.broadcasted_iota(i32, (160, 128), 1),
                   1.0, 0.0).astype(bf16)
    c_phi.wait()
    for d in range(DH):
        w3 = jnp.concatenate([wphi_ref[d], jnp.zeros((128 - DH, H), bf16)], axis=0)
        wc_ref[pl.ds(d, H, stride=DH), :] = lax.dot_general(eye, w3, NT, preferred_element_type=f32)
    c_part[0].start()
    c_part[2].start()
    afold = []
    for j in range(4):
        k0 = 128 * j
        kk = lax.broadcasted_iota(i32, (160, 256), 1) + k0
        hrow = 8 * j + (lax.broadcasted_iota(i32, (160, 256), 0) & 7)
        a = lax.dot_general(oh, wc_ref[k0:k0 + 256, :].astype(bf16), NT, preferred_element_type=f32)
        afold.append(jnp.where(hrow == ((kk * 3277) >> 16), a, 0.0).astype(bf16))

    def fold(part, j):
        def f():
            if j == 0:
                c_part[part].wait()
            c0 = part * D + 128 * j
            r = lax.dot_general(afold[j], _b(wqkv_ref[:, c0:c0 + 256]), NT, preferred_element_type=f32) * LOG2E
            r0 = (part * D + 160 * j) // 2
            wt_ref[r0:r0 + 80, :] = pltpu.bitcast(r.astype(bf16), u32)
        return f

    def vtrans(j):
        def f():
            if j == 0:
                c_part[2].wait()
            c0 = 2 * D + 128 * j
            wt_ref[c0 // 2:c0 // 2 + 64, :] = pltpu.bitcast(_b(wqkv_ref[:, c0:c0 + 128]).T, u32)
        return f

    for t in range(NW1, NTILE):
        x_copy(t).start()
    c_wo.start()
    c_w1.start()
    c_w2.start()
    kv_ref[...] = jnp.zeros(kv_ref.shape, f32)
    for j in range(4):
        fold(1, j)()
    late = [fold(0, j) for j in range(4)]
    late2 = [vtrans(j) for j in range(5)]

    rowi = lax.broadcasted_iota(i32, (48, 128), 0)
    coli = lax.broadcasted_iota(i32, (48, 128), 1)
    rhead = jnp.where(rowi < 40, jnp.where(rowi < 20, 0, 1), jnp.where(rowi < 44, 0, 1))
    chead = jnp.where(coli < 40, 0, jnp.where(coli < 80, 1, 2))
    kvmask = rhead == chead
    sub = lax.broadcasted_iota(i32, (8, T), 0)

    def finalize_kv(last):
        for g in range(G):
            kvb_ref[g] = pltpu.bitcast(jnp.where(kvmask, kv_ref[g], 0.0).astype(bf16), u32)
        if not last:
            kv_ref[...] = jnp.zeros(kv_ref.shape, f32)

    def ln_in(u):
        def f():
            y2_ref[hrows(u), :] = _ln(x_ref[rows(u), :].astype(f32))
        return f

    def wait_x(us):
        def f():
            for u in us:
                x_copy(u).wait()
        return f

    def softmax_store(p, j, dst, lead):
        p = [p[f * 8:(f + 1) * 8, :] for f in range(DH)]
        mx = _tree(jnp.maximum, p)
        mn = _tree(jnp.minimum, p)
        for sign in range(2):
            e = [jnp.exp2(v - mx) if sign == 0 else jnp.exp2(mn - v) for v in p]
            r = _rcp(_tree(jnp.add, e))
            for jj in range(DH // 2):
                w = _pack(e[2 * jj] * r, e[2 * jj + 1] * r)
                dst[lead, pl.ds(j * 160 + sign * 10 + jj, 8, stride=DH), :] = w

    def st_wz(t, n, pre=(), nxt=(), hold=None, pre2=()):
        nc = n * T // 128
        st = {}
        blocks = [(c, j) for c in range(nc) for j in range(4)]
        nb = len(blocks) // NSM

        def proj(part):
            def f():
                y = y2_ref[t * n * T // 2:(t + 1) * n * T // 2, :]
                for m in range(MS):
                    r0 = (part * D + m * (D // MS)) // 2
                    st[part, m] = lax.dot_general(_b(wt_ref[r0:r0 + D // MS // 2, :]), _b(y), NT, preferred_element_type=f32)
            return f

        def sm(part, i):
            def f():
                for c, j in blocks[i * nb:(i + 1) * nb]:
                    jm = j % (4 // MS)
                    pb = st[part, j // (4 // MS)][jm * 160:(jm + 1) * 160, c * 128:(c + 1) * 128]
                    if part == 1:
                        softmax_store(pb, j, phik_ref, c)
                    else:
                        softmax_store(pb, j, phiq_ref, t * nc + c)
            return f

        def kv(i):
            def f():
                for g in range(i * G // NKV, (i + 1) * G // NKV):
                    gm = g % (G // MS)
                    v = st[2, g // (G // MS)][gm * 40:gm * 40 + 40, :]
                    va = jnp.concatenate([v, jnp.ones((8, n * T), f32)], axis=0).astype(bf16)
                    pk = jnp.concatenate([_b(phik_ref[c, g * 40:(g + 1) * 40, :]) for c in range(nc)], axis=1)
                    r = lax.dot_general(va, pk, NT, preferred_element_type=f32)
                    kv_ref[g, :, 0:80] = kv_ref[g, :, 0:80] + r
            return f
        smk = [sm(1, i) for i in range(NSM)]
        smq = [sm(0, i) for i in range(NSM)]
        lns = [ln_in(u) for u in nxt]
        h = NSM // 2
        if hold is not None:
            hold.extend([proj(0)] + smq)
            return [proj(1)] + smk[:h] + [proj(2)] + smk[h:] + [kv(i) for i in range(NKV)]
        w = [wait_x(nxt)] if nxt else []
        kvs = [kv(i) for i in range(NKV)]
        return ([proj(1)] + smk[:h] + list(pre) + w + [proj(0)] + list(pre2) + smk[h:] + lns[:1]
                + [proj(2)] + smq[:h] + lns[1:] + kvs + smq[h:])

    def st_x(t, layer):
        NC = T // 128
        os_ = []

        def num(g0):
            def f():
                for g in range(g0, g0 + GPP):
                    pq = jnp.concatenate([_b(phiq_ref[t * NC + c, g * 40:(g + 1) * 40, :]) for c in range(NC)], axis=1)
                    n = jnp.dot(_b(kvb_ref[g])[:, 0:80], pq, preferred_element_type=f32)
                    r01 = _rcp(n[40:48] + 1e-6)
                    rsw = pltpu.roll(r01, 4, 0)
                    r0 = jnp.where(sub < 4, r01, rsw)
                    r1 = jnp.where(sub < 4, rsw, r01)
                    os_.extend([n[0:8] * r0, n[8:16] * r0, n[16:24] * r01, n[24:32] * r1, n[32:40] * r1])
            return f

        def fin():
            ot = jnp.concatenate(os_, axis=0).astype(bf16)
            a = lax.dot_general(ot, _b(wo_ref[...]), TN, preferred_element_type=f32)
            x = (x_ref[rows(t), :].astype(f32) if layer == 0 else xs_ref[rows(t), :]) + a
            xs_ref[rows(t), :] = x
            y1_ref[hrows(t), :] = _ln(x)
        return [num(g0) for g0 in range(0, G, GPP)] + [fin]

    def st_y(t, layer):
        st = {}
        chunks = [(c0, min(c0 + FC, F)) for c0 in range(0, F, FC)]

        def up(i):
            c0, c1 = chunks[i]
            h = lax.dot_general(_b(y1_ref[hrows(t), :]), _b(w1t_ref[c0 // 2:c1 // 2, :]), NT, preferred_element_type=f32)
            st[i] = h

        def down(i):
            c0, c1 = chunks[i]
            hh = 0.5 * st.pop(i)
            a = (hh + hh * jnp.tanh(hh)).astype(bf16)
            r = jnp.dot(a, _b(w2_ref[c0 // 2:c1 // 2, :]), preferred_element_type=f32)
            st["acc"] = (xs_ref[rows(t), :] if i == 0 else st["acc"]) + r

        def step(i):
            def f():
                if i == 0:
                    up(0)
                if i + 1 < len(chunks):
                    up(i + 1)
                down(i)
            return f

        def fin():
            x = st["acc"]
            if layer == 0:
                xs_ref[rows(t), :] = x
                y2_ref[hrows(t), :] = _ln(x)
            else:
                x_ref[rows(t), :] = x.astype(bf16)
                o_copy(t).start()
        return [step(i) for i in range(len(chunks))] + [fin]

    def run(stages, nt, held=()):
        ev = [(HT0 + k * HDT, -1, 0, k, p) for k, p in enumerate(held)]
        for si, (fn, start, dur) in enumerate(stages):
            for t in range(nt):
                ps = fn(t)
                for k, p in enumerate(ps):
                    ev.append((t + start + dur * (k + 0.5) / len(ps), si, t, k, p))
        ev.sort(key=lambda e: e[:4])
        for e in ev:
            e[4]()

    held1, held2 = [], []
    wait_x(range(NW1))()
    for u in range(NW1):
        ln_in(u)()
    n1 = NTILE // NW1
    run([(lambda t: st_wz(t, NW1, late if t == 0 else (),
                          range((t + 1) * NW1, (t + 2) * NW1) if t + 1 < n1 else (),
                          held1 if t == n1 - 1 else None,
                          late2 if t == 0 else ()), 0.0, 1.0)], n1)
    finalize_kv(False)
    c_wo.wait()
    c_w1.wait()
    c_w2.wait()
    run([(lambda t: st_x(t, 0), 0.0, XD), (lambda t: st_y(t, 0), XD + GAP, 1.0),
         (lambda t: st_wz(t, 1, hold=held2 if t == NTILE - 1 else None), XD + GAP + 1.0 + GAP2, 1.0)], NTILE, held1)
    finalize_kv(True)
    run([(lambda t: st_x(t, 1), 0.0, XD), (lambda t: st_y(t, 1), XD + GAP3, 1.0)], NTILE, held2)
    for t in range(NTILE):
        o_copy(t).wait()


@jax.jit
def pallas_interleave_layers__linear_kernel_hedgehog__dense_activation_silu__prompt_kernel(
        A_x, A_wqkv, A_w_phi, A_wo, B_x, B_w1, B_w2):
    NC = T // 128
    out = pl.pallas_call(
        kernel,
        out_shape=jax.ShapeDtypeStruct((S, D), bf16),
        in_specs=[pl.BlockSpec(memory_space=pl.ANY)] * 6,
        out_specs=pl.BlockSpec(memory_space=pl.ANY),
        scratch_shapes=[
            pltpu.VMEM((S, D), bf16),
            pltpu.VMEM((D // 2, 3 * D), u32),
            pltpu.VMEM((DH, DH, H), bf16),
            pltpu.VMEM((D // 2, D), u32),
            pltpu.VMEM((F // 2, D), u32),
            pltpu.VMEM((F // 2, D), u32),
            pltpu.VMEM((D + 24, 128), f32),
            pltpu.VMEM((S, D), f32),
            pltpu.VMEM((S // 2, D), u32),
            pltpu.VMEM((S // 2, D), u32),
            pltpu.VMEM((3 * D // 2, D), u32),
            pltpu.VMEM((S // 128, G * 40 + 24, 128), u32),
            pltpu.VMEM((NW1 * NC, G * 40 + 24, 128), u32),
            pltpu.VMEM((G, 48, 128), f32),
            pltpu.VMEM((G, 24, 128), u32),
            pltpu.SemaphoreType.DMA((7,)),
            pltpu.SemaphoreType.DMA((S // T,)),
            pltpu.SemaphoreType.DMA((S // T,)),
        ],
        compiler_params=pltpu.CompilerParams(vmem_limit_bytes=110 * 1024 * 1024, flags={'XLA_TPU_EVENLY_DISTRIBUTE_CRITICAL_NODES': True}),
    )(A_x.reshape(S, D), A_wqkv, jnp.transpose(A_w_phi, (1, 2, 0)), A_wo, B_w1.T, B_w2)
    return out.reshape(1, S, D)
```
